```python
import jax
import jax.numpy as jnp

def _softmax(x, axis=-1):
    return jax.nn.softmax(x, axis=axis)
def _gelu(x):
    return jax.nn.gelu(x, approximate=True)
def _silu(x):
    return jax.nn.silu(x)
def _sigmoid(x):
    return jax.nn.sigmoid(x)
def _layernorm(x, axis=-1, eps=1e-5):
    m = jnp.mean(x, axis=axis, keepdims=True)
    v = jnp.var(x, axis=axis, keepdims=True)
    return (x - m) / jnp.sqrt(v + eps)
def _scatter_add(tgt, idx, src, axis=0):
    return tgt.at[idx].add(src)
def _segment_sum(src, seg, n):
    return jax.ops.segment_sum(src, seg, n)
class _Rng:
    def __init__(self, key):
        self._k = key
    def _next(self):
        self._k, sub = jax.random.split(self._k)
        return sub
    def normal(self, shape):
        return jax.random.normal(self._next(), shape, dtype=jnp.bfloat16)
    def randint(self, lo, hi, shape):
        return jax.random.randint(self._next(), shape, lo, hi, dtype=jnp.int32)
    def uniform(self, shape, lo=0.0, hi=1.0):
        return jax.random.uniform(self._next(), shape, jnp.bfloat16, lo, hi)
    def permutation(self, n):
        return jax.random.permutation(self._next(), n)


kernel_name = 'recurrent_scan__mha_block_cached__moe_arch_mod__decode'

def setup_inputs():
    _rng = _Rng(jax.random.key(int.from_bytes(__import__("os").urandom(4), "little")))
    _w = (lambda a: (lambda t: t.astype(jnp.bfloat16) if jnp.issubdtype(t.dtype, jnp.floating) else t)(jnp.asarray(a)))
    def _A_setup():
        B, Sq, D = 2, 1, 512
        H, Sk, Dh = 32, 16384, 128
        return {
            "x": _w((lambda *s: _rng.normal(s) * 0.05)(B, Sq, D)),
            "k_cache": _w((lambda *s: _rng.normal(s) * 0.05)(B, H, Sk, Dh)),
            "v_cache": _w((lambda *s: _rng.normal(s) * 0.05)(B, H, Sk, Dh)),
            "wq": _w((lambda *s: _rng.normal(s) * 0.05)(D, H * Dh) * (D ** -0.5)),
            "wo": _w((lambda *s: _rng.normal(s) * 0.05)(H * Dh, D) * ((H * Dh) ** -0.5)),
        }
    _A_in = _A_setup()

    def _B_setup():
        B, S, D, F, C = 2, 1, 512, 1792, 1
        return {
            "x": _w((lambda *s: _rng.normal(s) * 0.05)(B, S, D)),
            "w_r": _w((lambda *s: _rng.normal(s) * 0.05)(D)),
            "w_gate": _w((lambda *s: _rng.normal(s) * 0.05)(D, F)),
            "w_up": _w((lambda *s: _rng.normal(s) * 0.05)(D, F)),
            "w_down": _w((lambda *s: _rng.normal(s) * 0.05)(F, D)),
        }
    _B_in = _B_setup()

    return {
        "A_x": _A_in["x"],
        "A_k_cache": _A_in["k_cache"],
        "A_v_cache": _A_in["v_cache"],
        "A_wq": _A_in["wq"],
        "A_wo": _A_in["wo"],
        "B_x": _B_in["x"],
        "B_w_r": _B_in["w_r"],
        "B_w_gate": _B_in["w_gate"],
        "B_w_up": _B_in["w_up"],
        "B_w_down": _B_in["w_down"],
    }

def reference(A_x, A_k_cache, A_v_cache, A_wq, A_wo, B_x, B_w_r, B_w_gate, B_w_up, B_w_down):
    def _A_ref(x, k_cache, v_cache, wq, wo):
        B, Sq, D = x.shape
        H, Dh = 32, 128
        q = (lambda x, *d: x.transpose(*d))((x @ wq).reshape(B, Sq, H, Dh), 0, 2, 1, 3)
        scores = jnp.einsum("bhqd,bhkd->bhqk", q, k_cache) * (Dh ** -0.5)
        p = _softmax(scores, axis=-1)
        o = jnp.einsum("bhqk,bhkd->bhqd", p, v_cache)
        return (lambda x, *d: x.transpose(*d))(o, 0, 2, 1, 3).reshape(B, Sq, H * Dh) @ wo

    def _B_ref(x, w_r, w_gate, w_up, w_down):
        B, S, D = x.shape
        C = 1
        r = x @ w_r
        idx = jnp.argsort(-r, axis=-1)[:, :C]
        idx_e = jnp.repeat(idx.reshape(B, C, 1), D, axis=2)
        x_sel = jnp.take_along_axis(x, idx_e, axis=1)
        g = _silu(x_sel @ w_gate)
        u = x_sel @ w_up
        y = (g * u) @ w_down
        r_sel = _sigmoid(jnp.take_along_axis(r, idx, axis=1))
        y = y * r_sel.reshape(B, C, 1)
        b_off = (jnp.arange(B) * S).reshape(B, 1)
        flat_idx = (idx + b_off).reshape(B * C)
        zero = (x * 0.0).reshape(B * S, D)
        upd = _scatter_add(zero, flat_idx, y.reshape(B * C, D), axis=0)
        return x + upd.reshape(B, S, D)

    x = A_x
    xn = _layernorm(x, axis=-1)
    s = _A_ref(xn, A_k_cache, A_v_cache, A_wq, A_wo)
    g = _silu(_B_ref(xn, B_w_r, B_w_gate, B_w_up, B_w_down))
    return x + s * g
```

```python
import functools

import jax
import jax.numpy as jnp
from jax import lax
import jax.experimental.pallas as pl
import jax.experimental.pallas.tpu as pltpu

F32, BF16 = jnp.float32, jnp.bfloat16
NT = (((1,), (1,)), ((), ()))
NN = (((1,), (0,)), ((), ()))


def make(BLK=256, HK=48, HV=0, NG=5, nobc=True, mode=0):
    B, D, H, S, DH = 2, 512, 32, 16384, 128
    GRP = 1024
    BPG = GRP // BLK
    TPB = BLK // 128
    GPH = S // GRP
    NGT = H * GPH
    AHEAD = NG - 1

    def kern(x_hbm, k_hbm, v_hbm, wq_hbm, wo_hbm, wr_hbm, wg_hbm, wu_hbm, wd_hbm, o_ref,
             kbuf, vbuf, xb, wq, wo, wr, wg, wu, wd, q_scr, s_scr, ksem, vsem, wsem):

        def start(hbm, buf, sem, b, grp, slot, j):
            HI = HK if hbm is k_hbm else HV
            row = pl.multiple_of(grp * GRP + j * BLK, BLK)
            if HI:
                pltpu.make_async_copy(hbm.at[b, pl.ds(row, HI)], buf.at[b, slot, j, pl.ds(0, HI)],
                                      sem.at[b, slot, j]).start(priority=0)
            pltpu.make_async_copy(hbm.at[b, pl.ds(pl.multiple_of(row + HI, 16), BLK - HI)],
                                  buf.at[b, slot, j, pl.ds(HI, BLK - HI)],
                                  sem.at[b, slot, j]).start(priority=1)

        def wait(buf, sem, b, slot, j):
            pltpu.make_async_copy(buf.at[b, slot, j], buf.at[b, slot, j], sem.at[b, slot, j]).wait()

        cp_x = pltpu.make_async_copy(x_hbm, xb, wsem.at[0])
        cp_wq = pltpu.make_async_copy(wq_hbm, wq, wsem.at[1])
        cp_rest = [pltpu.make_async_copy(s, d, wsem.at[2 + i]) for i, (s, d) in enumerate(
            ((wr_hbm, wr), (wg_hbm, wg), (wu_hbm, wu), (wd_hbm, wd), (wo_hbm, wo)))]
        cp_x.start(priority=0)
        cp_wq.start(priority=1)
        for g in range(AHEAD):
            for j in range(BPG):
                for b in range(B):
                    start(k_hbm, kbuf, ksem, b, g, g, j)
        for c in cp_rest:
            c.start(priority=1)

        sub = lax.broadcasted_iota(jnp.int32, (8, 128), 0)
        sub_d = lax.broadcasted_iota(jnp.int32, (8, D), 0)
        cp_x.wait()
        x2 = xb[...].astype(F32)
        x = jnp.where(sub_d == 0, x2[0:1], x2[1:2])
        mean = jnp.mean(x, axis=-1, keepdims=True)
        xc = x - mean
        var = jnp.mean(xc * xc, axis=-1, keepdims=True)
        xn = (xc / jnp.sqrt(var + 1e-5)).astype(BF16)
        cp_wq.wait()
        q = lax.dot_general(xn, wq[...], NN, preferred_element_type=F32)
        for h in range(H):
            qh = q[:, h * DH:(h + 1) * DH]
            for b in range(B):
                q_scr[b, h] = jnp.broadcast_to(qh[b:b + 1], (8, DH))

        scale = DH ** -0.5

        def group(gi, carry, h, m, do_k, do_v, k_next, v_next):
            mx, l, acc = (list(c) for c in carry)
            kg = h * GPH + gi
            vg = kg - GPH
            slot = lax.rem(kg, NG)
            nslot = lax.rem(kg + AHEAD, NG)
            if do_v:
                p = []
                for b in range(B):
                    pb = jnp.exp(s_scr[b, gi] - m[b])
                    l[b] = l[b] + pb
                    p.append(pb.astype(BF16))
            if do_k:
                qb = [q_scr[b, h].astype(BF16) for b in range(B)]
                s = [jnp.zeros((8, 128), F32)] * B
            def comp(b, j):
                for t in range(TPB):
                    if do_k:
                        r = lax.dot_general(qb[b], kbuf[b, slot, j, pl.ds(t * 128, 128)], NT,
                                            preferred_element_type=F32)
                        s[b] = jnp.where(sub == j * TPB + t, r, s[b])
                for t in range(TPB):
                    if do_v:
                        r = lax.dot_general(p[b], vbuf[b, slot, j, pl.ds(t * 128, 128)], NN,
                                            preferred_element_type=F32)
                        acc[b] = acc[b] + jnp.where(sub == j * TPB + t, r, 0.0)
            wk = lambda b, j: wait(kbuf, ksem, b, slot, j) if do_k else None
            wv = lambda b, j: wait(vbuf, vsem, b, slot, j) if do_v else None
            sk = lambda b, j: start(k_hbm, kbuf, ksem, b, kg + AHEAD, nslot, j) if k_next else None
            sv = lambda b, j: start(v_hbm, vbuf, vsem, b, vg + AHEAD, nslot, j) if v_next else None
            for j in range(BPG):
                if mode == 0:
                    for b in range(B):
                        wk(b, j); wv(b, j); sk(b, j); sv(b, j); comp(b, j)
                elif mode == 1:
                    for b in range(B):
                        wk(b, j); wv(b, j); sk(b, j); comp(b, j); sv(b, j)
                elif mode == 2:
                    for b in range(B):
                        wk(b, j); wv(b, j)
                    sk(0, j); sv(0, j); comp(0, j); comp(1, j); sk(1, j); sv(1, j)
                elif mode == 3:
                    for b in range(B):
                        wk(b, j); wv(b, j)
                    sk(0, j); sv(0, j); comp(0, j); sk(1, j); sv(1, j); comp(1, j)
            if do_k:
                for b in range(B):
                    sb = s[b] * scale
                    s_scr[b, gi] = sb
                    mx[b] = jnp.maximum(mx[b], sb)
            return tuple(mx), tuple(l), tuple(acc)

        def phase(h, m, do_k, do_v, tail_k, tail_v):
            zero = jnp.zeros((8, 128), F32)
            carry = ((jnp.full((8, 128), -jnp.inf, F32),) * B, (zero,) * B, (zero,) * B)
            carry = lax.fori_loop(
                0, GPH - AHEAD,
                functools.partial(group, h=h, m=m, do_k=do_k, do_v=do_v, k_next=do_k, v_next=do_v), carry)
            carry = lax.fori_loop(
                GPH - AHEAD, GPH,
                functools.partial(group, h=h, m=m, do_k=do_k, do_v=do_v, k_next=tail_k, v_next=tail_v), carry)
            mx, l, acc = carry
            m_new = m
            if do_k:
                m_new = tuple(
                    jnp.broadcast_to(jnp.max(jnp.max(mx[b], axis=0, keepdims=True), axis=1, keepdims=True), (8, 128))
                    for b in range(B))
            so = None
            if do_v:
                o = []
                for b in range(B):
                    lb = jnp.sum(jnp.sum(l[b], axis=0, keepdims=True), axis=1, keepdims=True)
                    o.append(jnp.sum(acc[b], axis=0, keepdims=True) / lb)
                o2 = jnp.where(sub == 0, o[0], o[1]).astype(BF16)
                so = lax.dot_general(o2, wo[pl.ds(pl.multiple_of((h - 1) * DH, DH), DH), :], NN,
                                     preferred_element_type=F32)
            return m_new, so

        m0 = (jnp.zeros((8, 128), F32),) * B
        m, _ = phase(0, m0, True, False, True, True)

        for c in cp_rest:
            c.wait()
        xnf = xn.astype(F32)
        r = jnp.sum(xnf * wr[...].astype(F32).reshape(1, D), axis=-1, keepdims=True)
        gate = lax.dot_general(xn, wg[...], NN, preferred_element_type=F32)
        up = lax.dot_general(xn, wu[...], NN, preferred_element_type=F32)
        hid = (gate * jax.nn.sigmoid(gate) * up).astype(BF16)
        y = lax.dot_general(hid, wd[...], NN, preferred_element_type=F32) * jax.nn.sigmoid(r)
        z = xnf + (xnf * 0.0 + y)
        g = z * jax.nn.sigmoid(z)

        def mid(h, c):
            m, sacc = c
            m, so = phase(h, m, True, True, True, True)
            return m, sacc + so

        m, sacc = lax.fori_loop(1, H - 1, mid, (m, jnp.zeros((8, D), F32)))
        m, so = phase(H - 1, m, True, True, False, True)
        sacc = sacc + so
        _, so = phase(H, m, False, True, False, False)
        sacc = sacc + so
        out = x + sacc * g
        o_ref[...] = out[0:B].astype(o_ref.dtype)

    def fn(A_x, A_k_cache, A_v_cache, A_wq, A_wo, B_x, B_w_r, B_w_gate, B_w_up, B_w_down, out_dtype=None):
        F = B_w_gate.shape[1]
        hbm = pl.BlockSpec(memory_space=pltpu.HBM)
        return pl.pallas_call(
            kern,
            in_specs=[hbm] * 9,
            out_specs=pl.BlockSpec(memory_space=pltpu.VMEM),
            out_shape=jax.ShapeDtypeStruct((B, D), out_dtype or A_x.dtype),
            scratch_shapes=[
                pltpu.VMEM((B, NG, BPG, BLK, DH), BF16),
                pltpu.VMEM((B, NG, BPG, BLK, DH), BF16),
                pltpu.VMEM((B, D), BF16),
                pltpu.VMEM(A_wq.shape, BF16),
                pltpu.VMEM(A_wo.shape, BF16),
                pltpu.VMEM(B_w_r.shape, BF16),
                pltpu.VMEM((D, F), BF16),
                pltpu.VMEM((D, F), BF16),
                pltpu.VMEM((F, D), BF16),
                pltpu.VMEM((B, H, 8, DH), F32),
                pltpu.VMEM((B, GPH, 8, 128), F32),
                pltpu.SemaphoreType.DMA((B, NG, BPG)),
                pltpu.SemaphoreType.DMA((B, NG, BPG)),
                pltpu.SemaphoreType.DMA((7,)),
            ],
            compiler_params=pltpu.CompilerParams(
                vmem_limit_bytes=64 * 1024 * 1024, disable_bounds_checks=nobc),
        )(A_x.reshape(B, D), A_k_cache.reshape(B, H * S, DH), A_v_cache.reshape(B, H * S, DH), A_wq, A_wo,
          B_w_r, B_w_gate, B_w_up, B_w_down).reshape(A_x.shape)

    return fn


@jax.jit
def pallas_recurrent_scan__mha_block_cached__moe_arch_mod__decode_kernel(
        A_x, A_k_cache, A_v_cache, A_wq, A_wo, B_x, B_w_r, B_w_gate, B_w_up, B_w_down):
    return make(mode=3)(A_x, A_k_cache, A_v_cache, A_wq, A_wo, B_x, B_w_r, B_w_gate, B_w_up, B_w_down)
```

```python
import functools

import jax
import jax.numpy as jnp
from jax import lax
import jax.experimental.pallas as pl
import jax.experimental.pallas.tpu as pltpu

F32, BF16 = jnp.float32, jnp.bfloat16
NT = (((1,), (1,)), ((), ()))
NN = (((1,), (0,)), ((), ()))


def make(DK=256, DV=256, HK=(0, 48), HV=(0, 0), NG=5, mode=3, nobc=True):
    B, D, H, S, DH = 2, 512, 32, 16384, 128
    BLK, BPG = 256, 4
    GRP = BLK * BPG
    GPH = S // GRP
    NGT = H * GPH
    AHEAD = NG - 1

    def kern(x_hbm, k_hbm, v_hbm, wq_hbm, wo_hbm, wr_hbm, wg_hbm, wu_hbm, wd_hbm, o_ref,
             kbuf, vbuf, xb, wq, wo, wr, wg, wu, wd, q_scr, s_scr, ksem, vsem, wsem):
        KS = (k_hbm, kbuf, ksem, DK, HK)
        VS = (v_hbm, vbuf, vsem, DV, HV)

        def copy(st, b, grp, slot, j, lo, hi):
            hbm, buf, sem, d, _ = st
            row = pl.multiple_of(grp * GRP + (j * BLK - d + lo), 16)
            return pltpu.make_async_copy(hbm.at[b, pl.ds(row, hi - lo)],
                                         buf.at[b, slot, j, pl.ds(lo, hi - lo)], sem.at[b, slot, j])

        def start(st, b, grp, slot, j):
            h0, h1 = st[4]
            if h1 > h0:
                copy(st, b, grp, slot, j, h0, h1).start(priority=0)
                if h0 > 0:
                    copy(st, b, grp, slot, j, 0, h0).start(priority=1)
                if h1 < BLK:
                    copy(st, b, grp, slot, j, h1, BLK).start(priority=1)
            else:
                copy(st, b, grp, slot, j, 0, BLK).start(priority=1)

        def wait(st, b, slot, j, lo=0, hi=BLK):
            if hi > lo:
                dst = st[1].at[b, slot, j, pl.ds(lo, hi - lo)]
                pltpu.make_async_copy(dst, dst, st[2].at[b, slot, j]).wait()

        def start_first(st, b):
            if st[3] < BLK:
                copy(st, b, 0, 0, 0, st[3], BLK).start(priority=1)

        def start_last(st, b):
            copy(st, b, NGT, NGT % NG, 0, 0, st[3]).start(priority=1)

        def tile(st, b, slot, nxt, j, t):
            buf, d = st[1], st[3]
            lo, hi = d + 128 * t, d + 128 * t + 128
            parts = []
            if lo < BLK:
                parts.append(buf[b, slot, j, pl.ds(lo, min(hi, BLK) - lo)])
            if hi > BLK:
                s2, j2 = (slot, j + 1) if j + 1 < BPG else (nxt, 0)
                l2 = max(lo, BLK) - BLK
                parts.append(buf[b, s2, j2, pl.ds(l2, hi - BLK - l2)])
            return parts[0] if len(parts) == 1 else jnp.concatenate(parts, axis=0)

        cp_x = pltpu.make_async_copy(x_hbm, xb, wsem.at[0])
        cp_wq = pltpu.make_async_copy(wq_hbm, wq, wsem.at[1])
        cp_rest = [pltpu.make_async_copy(s, d, wsem.at[2 + i]) for i, (s, d) in enumerate(
            ((wr_hbm, wr), (wg_hbm, wg), (wu_hbm, wu), (wd_hbm, wd), (wo_hbm, wo)))]
        cp_x.start(priority=0)
        cp_wq.start(priority=1)
        for g in range(AHEAD):
            for j in range(BPG):
                for b in range(B):
                    if g == 0 and j == 0:
                        start_first(KS, b)
                    else:
                        start(KS, b, g, g, j)
        for c in cp_rest:
            c.start(priority=1)

        sub = lax.broadcasted_iota(jnp.int32, (8, 128), 0)
        sub_d = lax.broadcasted_iota(jnp.int32, (8, D), 0)
        cp_x.wait()
        x2 = xb[...].astype(F32)
        x = jnp.where(sub_d == 0, x2[0:1], x2[1:2])
        mean = jnp.mean(x, axis=-1, keepdims=True)
        xc = x - mean
        var = jnp.mean(xc * xc, axis=-1, keepdims=True)
        xn = (xc / jnp.sqrt(var + 1e-5)).astype(BF16)
        cp_wq.wait()
        q = lax.dot_general(xn, wq[...], NN, preferred_element_type=F32)
        for h in range(H):
            qh = q[:, h * DH:(h + 1) * DH]
            for b in range(B):
                q_scr[b, h] = jnp.broadcast_to(qh[b:b + 1], (8, DH))

        scale = DH ** -0.5

        def group(gi, carry, h, m, do_k, do_v, k_next, v_next):
            mx, l, acc = (list(c) for c in carry)
            kg = h * GPH + gi
            vg = kg - GPH
            kslot, knxt, kpre = lax.rem(kg, NG), lax.rem(kg + 1, NG), lax.rem(kg + AHEAD, NG)
            off = (-GPH) % NG
            vslot, vnxt, vpre = lax.rem(kg + off, NG), lax.rem(kg + off + 1, NG), lax.rem(kg + off + AHEAD, NG)
            if do_v:
                p = []
                for b in range(B):
                    pb = jnp.exp(s_scr[b, gi] - m[b])
                    l[b] = l[b] + pb
                    p.append(pb.astype(BF16))
            if do_k:
                qb = [q_scr[b, h].astype(BF16) for b in range(B)]
                s = [jnp.zeros((8, 128), F32)] * B

            def comp(b, j):
                for t in range(2):
                    if do_k:
                        r = lax.dot_general(qb[b], tile(KS, b, kslot, knxt, j, t), NT, preferred_element_type=F32)
                        s[b] = jnp.where(sub == j * 2 + t, r, s[b])
                for t in range(2):
                    if do_v:
                        r = lax.dot_general(p[b], tile(VS, b, vslot, vnxt, j, t), NN, preferred_element_type=F32)
                        acc[b] = acc[b] + jnp.where(sub == j * 2 + t, r, 0.0)

            def wt(st, nxt_mode, on, slot, nxt, b, j):
                if not on:
                    return
                if j + 1 < BPG:
                    wait(st, b, slot, j + 1)
                elif nxt_mode == 'last':
                    pl.when(gi == GPH - 1)(lambda: wait(st, b, nxt, 0, 0, st[3]))
                    pl.when(gi < GPH - 1)(lambda: wait(st, b, nxt, 0))
                else:
                    wait(st, b, nxt, 0)

            def pf(st, nxt_mode, grp, pre, b, j):
                if nxt_mode == 'full' or (nxt_mode == 'first' and j > 0):
                    start(st, b, grp + AHEAD, pre, j)
                elif nxt_mode == 'first':
                    pl.when(gi == GPH - AHEAD)(lambda: start_first(st, b))
                    pl.when(gi > GPH - AHEAD)(lambda: start(st, b, grp + AHEAD, pre, j))
                elif nxt_mode == 'last' and j == 0:
                    pl.when(gi == GPH - AHEAD)(lambda: start_last(st, b))

            wk = functools.partial(wt, KS, k_next, do_k, kslot, knxt)
            wv = functools.partial(wt, VS, v_next, do_v, vslot, vnxt)
            sk = functools.partial(pf, KS, k_next, kg, kpre)
            sv = functools.partial(pf, VS, v_next, vg, vpre)
            for j in range(BPG):
                if mode == 0:
                    for b in range(B):
                        wk(b, j); wv(b, j); sk(b, j); sv(b, j); comp(b, j)
                elif mode == 1:
                    for b in range(B):
                        wk(b, j); wv(b, j); sk(b, j); comp(b, j); sv(b, j)
                elif mode == 2:
                    for b in range(B):
                        wk(b, j); wv(b, j)
                    sk(0, j); sv(0, j); comp(0, j); comp(1, j); sk(1, j); sv(1, j)
                elif mode == 3:
                    for b in range(B):
                        wk(b, j); wv(b, j)
                    sk(0, j); sv(0, j); comp(0, j); sk(1, j); sv(1, j); comp(1, j)
            if do_k:
                for b in range(B):
                    sb = s[b] * scale
                    s_scr[b, gi] = sb
                    mx[b] = jnp.maximum(mx[b], sb)
            return tuple(mx), tuple(l), tuple(acc)

        def phase(h, m, do_k, do_v, tail_k, tail_v):
            zero = jnp.zeros((8, 128), F32)
            carry = ((jnp.full((8, 128), -jnp.inf, F32),) * B, (zero,) * B, (zero,) * B)
            fl = lambda on: 'full' if on else 'none'
            if (fl(do_k), fl(do_v)) == (tail_k, tail_v):
                carry = lax.fori_loop(
                    0, GPH,
                    functools.partial(group, h=h, m=m, do_k=do_k, do_v=do_v, k_next=tail_k, v_next=tail_v), carry)
            else:
                carry = lax.fori_loop(
                    0, GPH - AHEAD,
                    functools.partial(group, h=h, m=m, do_k=do_k, do_v=do_v, k_next=fl(do_k), v_next=fl(do_v)), carry)
                carry = lax.fori_loop(
                    GPH - AHEAD, GPH,
                    functools.partial(group, h=h, m=m, do_k=do_k, do_v=do_v, k_next=tail_k, v_next=tail_v), carry)
            mx, l, acc = carry
            m_new = m
            if do_k:
                m_new = tuple(
                    jnp.broadcast_to(jnp.max(jnp.max(mx[b], axis=0, keepdims=True), axis=1, keepdims=True), (8, 128))
                    for b in range(B))
            so = None
            if do_v:
                o = []
                for b in range(B):
                    lb = jnp.sum(jnp.sum(l[b], axis=0, keepdims=True), axis=1, keepdims=True)
                    o.append(jnp.sum(acc[b], axis=0, keepdims=True) / lb)
                o2 = jnp.where(sub == 0, o[0], o[1]).astype(BF16)
                so = lax.dot_general(o2, wo[pl.ds(pl.multiple_of((h - 1) * DH, DH), DH), :], NN,
                                     preferred_element_type=F32)
            return m_new, so

        for b in range(B):
            wait(KS, b, 0, 0, DK, BLK)
        m0 = (jnp.zeros((8, 128), F32),) * B
        m, _ = phase(0, m0, True, False, 'full', 'first')

        for c in cp_rest:
            c.wait()
        xnf = xn.astype(F32)
        r = jnp.sum(xnf * wr[...].astype(F32).reshape(1, D), axis=-1, keepdims=True)
        gate = lax.dot_general(xn, wg[...], NN, preferred_element_type=F32)
        up = lax.dot_general(xn, wu[...], NN, preferred_element_type=F32)
        hid = (gate * jax.nn.sigmoid(gate) * up).astype(BF16)
        y = lax.dot_general(hid, wd[...], NN, preferred_element_type=F32) * jax.nn.sigmoid(r)
        z = xnf + (xnf * 0.0 + y)
        g = z * jax.nn.sigmoid(z)
        for b in range(B):
            wait(VS, b, 0, 0, DV, BLK)

        def mid(h, c):
            m, sacc = c
            m, so = phase(h, m, True, True, 'full', 'full')
            return m, sacc + so

        m, sacc = lax.fori_loop(1, H - 1, mid, (m, jnp.zeros((8, D), F32)))
        m, so = phase(H - 1, m, True, True, 'last', 'full')
        sacc = sacc + so
        _, so = phase(H, m, False, True, 'none', 'last')
        sacc = sacc + so
        out = x + sacc * g
        o_ref[...] = out[0:B].astype(o_ref.dtype)

    def fn(A_x, A_k_cache, A_v_cache, A_wq, A_wo, B_x, B_w_r, B_w_gate, B_w_up, B_w_down, out_dtype=None):
        F = B_w_gate.shape[1]
        hbm = pl.BlockSpec(memory_space=pltpu.HBM)
        return pl.pallas_call(
            kern,
            in_specs=[hbm] * 9,
            out_specs=pl.BlockSpec(memory_space=pltpu.VMEM),
            out_shape=jax.ShapeDtypeStruct((B, D), out_dtype or A_x.dtype),
            scratch_shapes=[
                pltpu.VMEM((B, NG, BPG, BLK, DH), BF16),
                pltpu.VMEM((B, NG, BPG, BLK, DH), BF16),
                pltpu.VMEM((B, D), BF16),
                pltpu.VMEM(A_wq.shape, BF16),
                pltpu.VMEM(A_wo.shape, BF16),
                pltpu.VMEM(B_w_r.shape, BF16),
                pltpu.VMEM((D, F), BF16),
                pltpu.VMEM((D, F), BF16),
                pltpu.VMEM((F, D), BF16),
                pltpu.VMEM((B, H, 8, DH), F32),
                pltpu.VMEM((B, GPH, 8, 128), F32),
                pltpu.SemaphoreType.DMA((B, NG, BPG)),
                pltpu.SemaphoreType.DMA((B, NG, BPG)),
                pltpu.SemaphoreType.DMA((7,)),
            ],
            compiler_params=pltpu.CompilerParams(
                vmem_limit_bytes=64 * 1024 * 1024, disable_bounds_checks=nobc),
        )(A_x.reshape(B, D), A_k_cache.reshape(B, H * S, DH), A_v_cache.reshape(B, H * S, DH), A_wq, A_wo,
          B_w_r, B_w_gate, B_w_up, B_w_down).reshape(A_x.shape)

    return fn


@jax.jit
def pallas_recurrent_scan__mha_block_cached__moe_arch_mod__decode_kernel(
        A_x, A_k_cache, A_v_cache, A_wq, A_wo, B_x, B_w_r, B_w_gate, B_w_up, B_w_down):
    return make(128,64,(240,256),(240,256),NG=4)(A_x, A_k_cache, A_v_cache, A_wq, A_wo, B_x, B_w_r, B_w_gate, B_w_up, B_w_down)
```

```python
import functools

import jax
import jax.numpy as jnp
from jax import lax
import jax.experimental.pallas as pl
import jax.experimental.pallas.tpu as pltpu

F32, BF16 = jnp.float32, jnp.bfloat16
NT = (((1,), (1,)), ((), ()))
NN = (((1,), (0,)), ((), ()))


def make(DK=128, DV=64, HI=16, RING=8, AHEAD=7, HA=3, HS=2, Q0=4, G=2, nobc=False, **cp):
    B, D, H, S, DH, F = 2, 512, 32, 16384, 128, 1792
    U = B * HS
    HP = H // HS
    BLK = 256
    NB = S // BLK
    NP = HP * NB
    HA = HA or AHEAD
    WS = 32
    NQ = 16

    def kern(x_hbm, k_hbm, v_hbm, wq_hbm, wo_hbm, wr_hbm, wg_hbm, wu_hbm, wd_hbm, o_ref,
             kbuf, vbuf, xb, wq, wo, wr, wg, wu, wd, q_scr, s_scr, p_scr, sems, wsem):
        KS = (k_hbm, kbuf, sems, DK)
        VS = (v_hbm, vbuf, sems, DV)

        def copy(st, u, n, lo, hi):
            hbm, buf, sem, d = st
            slot = n % RING
            row = n * BLK + (lo - d)
            if not isinstance(row, int):
                row = pl.multiple_of(row, 16)
            return pltpu.make_async_copy(hbm.at[u, pl.ds(row, hi - lo)],
                                         buf.at[u, slot, pl.ds(lo, hi - lo)], sem.at[u // G, slot])

        def start_lo(st, u, n, lo=0):
            copy(st, u, n, lo, BLK - HI).start(priority=1)

        def start_hi(st, u, n):
            copy(st, u, n, BLK - HI, BLK).start(priority=0)

        def wait(st, u, n, lo=0, hi=BLK):
            dst = st[1].at[u, n % RING, pl.ds(lo, hi - lo)]
            pltpu.make_async_copy(dst, dst, st[2].at[u // G, n % RING]).wait()

        def tile(st, u, m, t):
            buf, d = st[1], st[3]
            lo, hi = d + 128 * t, d + 128 * t + 128
            parts = []
            if lo < BLK:
                parts.append(buf[u, m % RING, pl.ds(lo, min(hi, BLK) - lo)])
            if hi > BLK:
                l2 = max(lo, BLK) - BLK
                parts.append(buf[u, (m + 1) % RING, pl.ds(l2, hi - BLK - l2)])
            return parts[0] if len(parts) == 1 else jnp.concatenate(parts, axis=0)

        def start_w(src, dst, sem, row, rows):
            cols = dst.shape[1]
            if not isinstance(row, int):
                row = pl.multiple_of(row, 8)
            if cols > 512:
                ih, il = (pl.ds(row, rows), pl.ds(cols - 256, 256)), (pl.ds(row, rows), pl.ds(0, cols - 256))
            else:
                ih, il = (pl.ds(row + (rows - 8), 8),), (pl.ds(row, rows - 8),)
            pltpu.make_async_copy(src.at[ih], dst.at[ih], sem).start(priority=0)
            pltpu.make_async_copy(src.at[il], dst.at[il], sem).start(priority=1)

        def start_q(c):
            for i in range(4):
                start_w(wq_hbm, wq, wsem, 128 * i + 8 * c, 8)

        def start_k0(n):
            for u in range(U):
                if n <= HA:
                    start_hi(KS, u, n)
                start_lo(KS, u, n, DK if n == 0 else 0)

        cp_x = pltpu.make_async_copy(x_hbm, xb, wsem)
        cp_r = pltpu.make_async_copy(wr_hbm, wr, wsem)
        cp_x.start(priority=0)
        todo = [functools.partial(start_q, c) for c in range(NQ)]
        todo += [functools.partial(start_k0, n) for n in range(AHEAD + 1 if AHEAD + 1 < RING else AHEAD)]
        for f in todo[:Q0]:
            f()
        todo = todo[Q0:]

        sub = lax.broadcasted_iota(jnp.int32, (8, 128), 0)
        sub_d = lax.broadcasted_iota(jnp.int32, (8, D), 0)
        for c in range(NQ):
            part = wq.at[pl.ds(0, D // NQ)]
            pltpu.make_async_copy(part, part, wsem).wait()
            for f in todo[c * len(todo) // NQ:(c + 1) * len(todo) // NQ]:
                f()
        cp_x.wait()
        cp_r.start(priority=0)
        x2 = xb[...].astype(F32)
        x = jnp.where(sub_d == 0, x2[0:1], x2[1:2])
        mean = jnp.mean(x, axis=-1, keepdims=True)
        xc = x - mean
        var = jnp.mean(xc * xc, axis=-1, keepdims=True)
        xn = (xc / jnp.sqrt(var + 1e-5)).astype(BF16)
        scale = DH ** -0.5
        LA = AHEAD + 1 if AHEAD + 1 < RING else AHEAD

        def step(i, acc, h, do_k, do_v, k_lo, k_hi, v_lo, v_hi, k_wait, v_wait, weights):
            acc = list(acc)
            mk = h * NB + i
            mv = mk - NB
            rows = sub - (i % 4) * 2

            def comp(u):
                if do_k:
                    qb = q_scr[u].astype(BF16)
                    s = s_scr[u, i // 4]
                    for t in range(2):
                        r = lax.dot_general(qb, tile(KS, u, mk, t), NT, preferred_element_type=F32)
                        s = jnp.where(rows == t, r, s)
                    s_scr[u, i // 4] = s
                if do_v:
                    pb = p_scr[u, i // 4].astype(BF16)
                    for t in range(2):
                        r = lax.dot_general(pb, tile(VS, u, mv, t), NN, preferred_element_type=F32)
                        acc[u] = acc[u] + jnp.where(rows == t, r, 0.0)

            def wt(st, kind, m, u):
                if kind == 'full':
                    wait(st, u, m + 1)
                elif kind == 'last':
                    wait(st, u, m + 1, 0, st[3])
                elif kind == 'first':
                    wait(st, u, 0, st[3], BLK)

            def pf(st, lo, hi, m, u):
                if hi == 'full':
                    start_hi(st, u, m + min(HA + 1, LA))
                if lo == 'full':
                    start_lo(st, u, m + LA)
                elif lo == 'first':
                    start_lo(st, u, 0, st[3])
                elif lo == 'last':
                    copy(st, u, NP, 0, st[3]).start(priority=1)

            def pw(u):
                if not weights:
                    return
                if u == 0:
                    start_w(wo_hbm, wo, wsem, 64 * i, 64)
                elif u == 1:
                    start_w(wg_hbm, wg, wsem, 16 * i, 16)
                elif u == 2:
                    start_w(wo_hbm, wo, wsem, 64 * i + 2048, 64)
                elif u == 3:
                    start_w(wu_hbm, wu, wsem, 16 * i, 16)
                    start_w(wd_hbm, wd, wsem, 56 * i, 56)

            for u0 in range(0, U, G):
                for u in range(u0, u0 + G):
                    wt(KS, k_wait, mk, u)
                    wt(VS, v_wait, mv, u)
                for u in range(u0, u0 + G):
                    pf(KS, k_lo, k_hi, mk, u)
                    pf(VS, v_lo, v_hi, mv, u)
                    pw(u)
                    comp(u)
            return tuple(acc)

        def kinds(h, i):
            def one(m):
                on = 0 <= m < NP
                n_lo, n_hi = m + LA, m + min(HA + 1, LA)
                lo = 'first' if n_lo == 0 else 'last' if n_lo == NP else 'full' if 0 < n_lo < NP else None
                hi = 'full' if 0 <= n_hi < NP else None
                w = 'first' if m + 1 == 0 else None if not on else 'last' if m + 1 == NP else 'full'
                return on, lo, hi, w
            k, v = one(h * NB + i), one(h * NB + i - NB)
            return dict(do_k=k[0], do_v=v[0], k_lo=k[1], k_hi=k[2], v_lo=v[1], v_hi=v[2], k_wait=k[3], v_wait=v[3],
                        weights=h == 0 and i < WS)

        def phase(h, h_static, l):
            do_k, do_v = h_static < HP, h_static > 0
            if do_k:
                for i in range(HS):
                    col = (i * HP + h) * DH
                    if not isinstance(col, int):
                        col = pl.multiple_of(col, DH)
                    q = lax.dot_general(xn, wq[:, pl.ds(col, DH)], NN, preferred_element_type=F32)
                    for b in range(B):
                        q_scr[b * HS + i] = jnp.broadcast_to(q[b:b + 1], (8, DH))
            acc = (jnp.zeros((8, 128), F32),) * U
            i0 = 0
            while i0 < NB:
                kw, i1 = kinds(h_static, i0), i0 + 1
                while i1 < NB and kinds(h_static, i1) == kw:
                    i1 += 1
                body = functools.partial(step, h=h, **kw)
                acc = body(i0, acc) if i1 == i0 + 1 else lax.fori_loop(i0, i1, body, acc)
                i0 = i1
            l_new = l
            if do_k:
                l_new = []
                for u in range(U):
                    sc = s_scr[u] * scale
                    m = jnp.max(jnp.max(jnp.max(sc, axis=0), axis=0, keepdims=True), axis=1, keepdims=True)
                    p = jnp.exp(sc - m)
                    p_scr[u] = p
                    l_new.append(jnp.sum(p, axis=0))
                l_new = tuple(l_new)
            so = None
            if do_v:
                o = []
                for u in range(U):
                    lu = jnp.sum(jnp.sum(l[u], axis=0, keepdims=True), axis=1, keepdims=True)
                    o.append(jnp.sum(acc[u], axis=0, keepdims=True) / lu)
                for i in range(HS):
                    o2 = jnp.where(sub == 0, o[i], o[HS + i]).astype(BF16)
                    row = (i * HP + h - 1) * DH
                    if not isinstance(row, int):
                        row = pl.multiple_of(row, DH)
                    r = lax.dot_general(o2, wo[pl.ds(row, DH), :], NN, preferred_element_type=F32)
                    so = r if so is None else so + r
            return l_new, so

        s_scr[...] = jnp.zeros(s_scr.shape, F32)
        for u in range(U):
            wait(KS, u, 0, DK, BLK)
        l, _ = phase(0, 0, None)

        cp_r.wait()
        for i, w in enumerate((wo, wg, wu, wd)):
            pltpu.make_async_copy(w, w, wsem).wait()
        xnf = xn.astype(F32)
        r = jnp.sum(xnf * wr[...].astype(F32).reshape(1, D), axis=-1, keepdims=True)
        gate = lax.dot_general(xn, wg[...], NN, preferred_element_type=F32)
        up = lax.dot_general(xn, wu[...], NN, preferred_element_type=F32)
        hid = (gate * jax.nn.sigmoid(gate) * up).astype(BF16)
        y = lax.dot_general(hid, wd[...], NN, preferred_element_type=F32) * jax.nn.sigmoid(r)
        z = xnf + (xnf * 0.0 + y)
        g = z * jax.nn.sigmoid(z)

        def mid(h, c):
            l, sacc = c
            l, so = phase(h, 1, l)
            return l, sacc + so

        l, sacc = lax.fori_loop(1, HP - 1, mid, (l, jnp.zeros((8, D), F32)))
        l, so = phase(HP - 1, HP - 1, l)
        sacc = sacc + so
        _, so = phase(HP, HP, l)
        sacc = sacc + so
        out = x + sacc * g
        o_ref[...] = out[0:B].astype(o_ref.dtype)

    def fn(A_x, A_k_cache, A_v_cache, A_wq, A_wo, B_x, B_w_r, B_w_gate, B_w_up, B_w_down, out_dtype=None):
        hbm = pl.BlockSpec(memory_space=pltpu.HBM)
        return pl.pallas_call(
            kern,
            in_specs=[hbm] * 9,
            out_specs=pl.BlockSpec(memory_space=pltpu.VMEM),
            out_shape=jax.ShapeDtypeStruct((B, D), out_dtype or A_x.dtype),
            scratch_shapes=[
                pltpu.VMEM((U, RING, BLK, DH), BF16),
                pltpu.VMEM((U, RING, BLK, DH), BF16),
                pltpu.VMEM((B, D), BF16),
                pltpu.VMEM(A_wq.shape, BF16),
                pltpu.VMEM(A_wo.shape, BF16),
                pltpu.VMEM(B_w_r.shape, BF16),
                pltpu.VMEM((D, F), BF16),
                pltpu.VMEM((D, F), BF16),
                pltpu.VMEM((F, D), BF16),
                pltpu.VMEM((U, 8, DH), F32),
                pltpu.VMEM((U, S // 1024, 8, 128), F32),
                pltpu.VMEM((U, S // 1024, 8, 128), F32),
                pltpu.SemaphoreType.DMA((U // G, RING)),
                pltpu.SemaphoreType.DMA(()),
            ],
            compiler_params=pltpu.CompilerParams(
                vmem_limit_bytes=64 * 1024 * 1024, disable_bounds_checks=nobc, **cp),
        )(A_x.reshape(B, D), A_k_cache.reshape(U, HP * S, DH), A_v_cache.reshape(U, HP * S, DH), A_wq, A_wo,
          B_w_r, B_w_gate, B_w_up, B_w_down).reshape(A_x.shape)

    return fn


@jax.jit
def pallas_recurrent_scan__mha_block_cached__moe_arch_mod__decode_kernel(
        A_x, A_k_cache, A_v_cache, A_wq, A_wo, B_x, B_w_r, B_w_gate, B_w_up, B_w_down):
    return make(G=4)(A_x, A_k_cache, A_v_cache, A_wq, A_wo, B_x, B_w_r, B_w_gate, B_w_up, B_w_down)
```

```python
import functools

import jax
import jax.numpy as jnp
from jax import lax
import jax.experimental.pallas as pl
import jax.experimental.pallas.tpu as pltpu

F32, BF16 = jnp.float32, jnp.bfloat16
_NN = (((1,), (0,)), ((), ()))
_NT = (((1,), (1,)), ((), ()))

HS = 2
BLK = 256
HI = 16
RING = 8
LO_AHEAD = 7
HI_AHEAD = 4
K_SHIFT, V_SHIFT = 128, 64
W_STEPS = 32
Q_CHUNKS = 16
Q_FIRST = 5


def _dot(a, b, dims=_NN):
    return lax.dot_general(a, b, dims, preferred_element_type=F32)


def _aligned(i, n):
    return i if isinstance(i, int) else pl.multiple_of(i, n)


def _kernel(x_hbm, k_hbm, v_hbm, wq_hbm, wo_hbm, wr_hbm, wg_hbm, wu_hbm, wd_hbm, o_ref,
            kbuf, vbuf, xb, wq, wo, wr, wg, wu, wd, q_scr, s_scr, p_scr, sems, wsem, *, seq):
    B, D = xb.shape
    F = wd.shape[0]
    U, stream_rows, DH = k_hbm.shape
    HP = stream_rows // seq
    NB = seq // BLK
    NP = HP * NB
    K = (k_hbm, kbuf, K_SHIFT)
    V = (v_hbm, vbuf, V_SHIFT)

    def start(st, u, n, lo, hi, priority):
        hbm, buf, shift = st
        pltpu.make_async_copy(
            hbm.at[u, pl.ds(_aligned(n * BLK + (lo - shift), 16), hi - lo)],
            buf.at[u, n % RING, pl.ds(lo, hi - lo)], sems.at[n % RING]).start(priority=priority)

    def wait(st, u, n, lo, hi):
        dst = st[1].at[u, n % RING, pl.ds(lo, hi - lo)]
        pltpu.make_async_copy(dst, dst, sems.at[n % RING]).wait()

    def tile(st, u, m, t):
        _, buf, shift = st
        lo, hi = shift + 128 * t, shift + 128 * (t + 1)
        parts = []
        if lo < BLK:
            parts.append(buf[u, m % RING, pl.ds(lo, min(hi, BLK) - lo)])
        if hi > BLK:
            lo = max(lo, BLK)
            parts.append(buf[u, (m + 1) % RING, pl.ds(lo - BLK, hi - lo)])
        return parts[0] if len(parts) == 1 else jnp.concatenate(parts, axis=0)

    def plan(m):
        def rows(n, lo, hi, shift):
            if n == 0:
                lo = max(lo, shift)
            if n == NP:
                hi = min(hi, shift)
            return (lo, hi) if 0 <= n <= NP and lo < hi else None
        return lambda shift: (0 <= m < NP,
                              rows(m + 1, 0, BLK, shift),
                              rows(m + HI_AHEAD, BLK - HI, BLK, shift),
                              rows(m + LO_AHEAD, 0, BLK - HI, shift))

    def start_weight(src, dst, row, n):
        cols = dst.shape[1]
        row = _aligned(row, 8)
        if cols > 512:
            small, bulk = (pl.ds(row, n), pl.ds(cols - 256, 256)), (pl.ds(row, n), pl.ds(0, cols - 256))
        else:
            small, bulk = (pl.ds(row + (n - 8), 8),), (pl.ds(row, n - 8),)
        pltpu.make_async_copy(src.at[small], dst.at[small], wsem).start(priority=0)
        pltpu.make_async_copy(src.at[bulk], dst.at[bulk], wsem).start(priority=1)

    def start_wq(c):
        n = D // (4 * Q_CHUNKS)
        for i in range(4):
            start_weight(wq_hbm, wq, i * (D // 4) + c * n, n)

    def start_weights(i, u):
        n = wo.shape[0] // (2 * W_STEPS)
        if u == 0:
            start_weight(wo_hbm, wo, n * i, n)
        elif u == 1:
            start_weight(wg_hbm, wg, (D // W_STEPS) * i, D // W_STEPS)
        elif u == 2:
            start_weight(wo_hbm, wo, n * (i + W_STEPS), n)
        else:
            start_weight(wu_hbm, wu, (D // W_STEPS) * i, D // W_STEPS)
            start_weight(wd_hbm, wd, (F // W_STEPS) * i, F // W_STEPS)

    def start_first_k(n):
        for u in range(U):
            if n < HI_AHEAD:
                start(K, u, n, BLK - HI, BLK, 0)
            start(K, u, n, K_SHIFT if n == 0 else 0, BLK - HI, 1)

    cp_x = pltpu.make_async_copy(x_hbm, xb, wsem)
    cp_r = pltpu.make_async_copy(wr_hbm, wr, wsem)
    cp_x.start()
    for c in range(Q_FIRST):
        start_wq(c)
    s_scr[...] = jnp.zeros(s_scr.shape, F32)
    todo = [functools.partial(start_wq, c) for c in range(Q_FIRST, Q_CHUNKS)]
    todo += [functools.partial(start_first_k, n) for n in range(LO_AHEAD)]
    for c in range(Q_CHUNKS):
        chunk = wq.at[pl.ds(0, D // Q_CHUNKS)]
        pltpu.make_async_copy(chunk, chunk, wsem).wait()
        for f in todo[c * len(todo) // Q_CHUNKS:(c + 1) * len(todo) // Q_CHUNKS]:
            f()
    cp_x.wait()
    cp_r.start()

    sub = lax.broadcasted_iota(jnp.int32, (8, DH), 0)
    x2 = xb[...].astype(F32)
    x = jnp.where(lax.broadcasted_iota(jnp.int32, (8, D), 0) == 0, x2[0:1], x2[1:2])
    xc = x - jnp.mean(x, axis=-1, keepdims=True)
    var = jnp.mean(xc * xc, axis=-1, keepdims=True)
    xn = (xc / jnp.sqrt(var + 1e-5)).astype(BF16)

    def step(i, acc, h, k_plan, v_plan, weights):
        acc = list(acc)
        mk = h * NB + i
        streams = ((K, mk, k_plan), (V, mk - NB, v_plan))
        reg, row = i // 4, sub - (i % 4) * 2
        for u in range(U):
            for st, m, (_, rows, _, _) in streams:
                if rows:
                    wait(st, u, m + 1, *rows)
        for u in range(U):
            for st, m, (_, _, hi_rows, lo_rows) in streams:
                if lo_rows:
                    start(st, u, m + LO_AHEAD, *lo_rows, 1)
                if hi_rows:
                    start(st, u, m + HI_AHEAD, *hi_rows, 0)
            if weights:
                start_weights(i, u)
            if k_plan[0]:
                q = q_scr[u].astype(BF16)
                s = s_scr[u, reg]
                for t in range(2):
                    s = jnp.where(row == t, _dot(q, tile(K, u, mk, t), _NT), s)
                s_scr[u, reg] = s
            if v_plan[0]:
                p = p_scr[u, reg].astype(BF16)
                for t in range(2):
                    acc[u] = acc[u] + jnp.where(row == t, _dot(p, tile(V, u, mk - NB, t)), 0.0)
        return tuple(acc)

    def phase(h, like, denom):
        def schedule(i):
            return dict(k_plan=plan(like * NB + i)(K_SHIFT), v_plan=plan((like - 1) * NB + i)(V_SHIFT),
                        weights=like == 0 and i < W_STEPS)

        if like < HP:
            for j in range(HS):
                q = _dot(xn, wq[:, pl.ds(_aligned((j * HP + h) * DH, DH), DH)])
                for b in range(B):
                    q_scr[b * HS + j] = jnp.broadcast_to(q[b:b + 1], (8, DH))
        acc = (jnp.zeros((8, DH), F32),) * U
        lo = 0
        while lo < NB:
            hi = lo + 1
            while hi < NB and schedule(hi) == schedule(lo):
                hi += 1
            body = functools.partial(step, h=h, **schedule(lo))
            acc = body(lo, acc) if hi == lo + 1 else lax.fori_loop(lo, hi, body, acc)
            lo = hi
        new_denom = None
        if like < HP:
            new_denom = []
            for u in range(U):
                s = s_scr[u] * (DH ** -0.5)
                top = jnp.max(jnp.max(jnp.max(s, axis=0), axis=0, keepdims=True), axis=1, keepdims=True)
                p = jnp.exp(s - top)
                p_scr[u] = p
                new_denom.append(jnp.sum(p, axis=0))
            new_denom = tuple(new_denom)
        proj = 0.0
        if like > 0:
            o = [jnp.sum(acc[u], axis=0, keepdims=True)
                 / jnp.sum(jnp.sum(denom[u], axis=0, keepdims=True), axis=1, keepdims=True)
                 for u in range(U)]
            for j in range(HS):
                rows = jnp.where(sub == 0, o[j], o[HS + j]).astype(BF16)
                proj = proj + _dot(rows, wo[pl.ds(_aligned((j * HP + h - 1) * DH, DH), DH), :])
        return new_denom, proj

    for u in range(U):
        wait(K, u, 0, K_SHIFT, BLK)
    denom, _ = phase(0, 0, None)

    cp_r.wait()
    for w in (wo, wg, wu, wd):
        pltpu.make_async_copy(w, w, wsem).wait()
    xf = xn.astype(F32)
    r = jnp.sum(xf * wr[...].astype(F32).reshape(1, D), axis=-1, keepdims=True)
    gate = _dot(xn, wg[...])
    hidden = (gate * jax.nn.sigmoid(gate) * _dot(xn, wu[...])).astype(BF16)
    y = _dot(hidden, wd[...]) * jax.nn.sigmoid(r)
    z = xf + (xf * 0.0 + y)
    g = z * jax.nn.sigmoid(z)

    def middle(h, carry):
        denom, proj = phase(h, 1, carry[0])
        return denom, carry[1] + proj

    denom, attn = lax.fori_loop(1, HP - 1, middle, (denom, jnp.zeros((8, D), F32)))
    for h in (HP - 1, HP):
        denom, proj = phase(h, h, denom)
        attn = attn + proj
    o_ref[...] = (x + attn * g)[0:B].astype(o_ref.dtype)


@jax.jit
def pallas_recurrent_scan__mha_block_cached__moe_arch_mod__decode_kernel(
    A_x: jax.Array,
    A_k_cache: jax.Array,
    A_v_cache: jax.Array,
    A_wq: jax.Array,
    A_wo: jax.Array,
    B_x: jax.Array,
    B_w_r: jax.Array,
    B_w_gate: jax.Array,
    B_w_up: jax.Array,
    B_w_down: jax.Array,
):
    del B_x
    B, H, S, DH = A_k_cache.shape
    D = A_x.shape[-1]
    U = B * HS
    assert (B, HS, DH) == (2, 2, 128) and A_x.shape[1] == 1
    assert H // HS >= 3 and S % 1024 == 0 and S // BLK >= W_STEPS and (S // BLK) % RING == 0

    def vmem_like(a):
        return pltpu.VMEM(a.shape, a.dtype)

    out = pl.pallas_call(
        functools.partial(_kernel, seq=S),
        in_specs=[pl.BlockSpec(memory_space=pltpu.HBM)] * 9,
        out_specs=pl.BlockSpec(memory_space=pltpu.VMEM),
        out_shape=jax.ShapeDtypeStruct((B, D), A_x.dtype),
        scratch_shapes=[
            pltpu.VMEM((U, RING, BLK, DH), A_k_cache.dtype),
            pltpu.VMEM((U, RING, BLK, DH), A_v_cache.dtype),
            pltpu.VMEM((B, D), A_x.dtype),
            vmem_like(A_wq),
            vmem_like(A_wo),
            vmem_like(B_w_r),
            vmem_like(B_w_gate),
            vmem_like(B_w_up),
            vmem_like(B_w_down),
            pltpu.VMEM((U, 8, DH), F32),
            pltpu.VMEM((U, S // 1024, 8, 128), F32),
            pltpu.VMEM((U, S // 1024, 8, 128), F32),
            pltpu.SemaphoreType.DMA((RING,)),
            pltpu.SemaphoreType.DMA(()),
        ],
        compiler_params=pltpu.CompilerParams(vmem_limit_bytes=48 * 1024 * 1024),
    )(A_x.reshape(B, D), A_k_cache.reshape(U, -1, DH), A_v_cache.reshape(U, -1, DH),
      A_wq, A_wo, B_w_r, B_w_gate, B_w_up, B_w_down)
    return out.reshape(A_x.shape)
```
